```python
import os as _os
_os.environ.setdefault("JAX_PLATFORMS", "cpu")
import jax
import jax.numpy as jnp

def _softmax(x, axis=-1):
    return jax.nn.softmax(x, axis=axis)
def _gelu(x):
    return jax.nn.gelu(x, approximate=True)
def _silu(x):
    return jax.nn.silu(x)
def _sigmoid(x):
    return jax.nn.sigmoid(x)
def _layernorm(x, axis=-1, eps=1e-5):
    m = jnp.mean(x, axis=axis, keepdims=True)
    v = jnp.var(x, axis=axis, keepdims=True)
    return (x - m) / jnp.sqrt(v + eps)
def _scatter_add(tgt, idx, src, axis=0):
    return tgt.at[idx].add(src)
def _segment_sum(src, seg, n):
    return jax.ops.segment_sum(src, seg, n)
class _Rng:
    def __init__(self, key):
        self._k = key
    def _next(self):
        self._k, sub = jax.random.split(self._k)
        return sub
    def normal(self, shape):
        return jax.random.normal(self._next(), shape, dtype=jnp.bfloat16)
    def randint(self, lo, hi, shape):
        return jax.random.randint(self._next(), shape, lo, hi, dtype=jnp.int32)
    def uniform(self, shape, lo=0.0, hi=1.0):
        return jax.random.uniform(self._next(), shape, jnp.bfloat16, lo, hi)
    def permutation(self, n):
        return jax.random.permutation(self._next(), n)


kernel_name = 'standalone__gqa_block_cached__near_ridge'

def setup_inputs():
    _rng = _Rng(jax.random.key(int.from_bytes(__import__("os").urandom(4), "little")))
    _w = (lambda a: (lambda t: t.astype(jnp.bfloat16) if jnp.issubdtype(t.dtype, jnp.floating) else t)(jnp.asarray(a)))
    B, Sq, D = 8, 64, 512
    Hq, Hkv, Sk, Dh = 32, 8, 64, 128
    assert Hq % Hkv == 0, (Hq, Hkv)
    return {
        "x": _w((lambda *s: _rng.normal(s) * 0.8)(B, Sq, D)),
        "k_cache": _w((lambda *s: _rng.normal(s) * 0.8)(B, Hkv, Sk, Dh)),
        "v_cache": _w((lambda *s: _rng.normal(s) * 0.05)(B, Hkv, Sk, Dh)),
        "wq": _w((lambda *s: _rng.normal(s) * 0.8)(D, Hq * Dh) * (D ** -0.5)),
        "wo": _w((lambda *s: _rng.normal(s) * 0.05)(Hq * Dh, D) * ((Hq * Dh) ** -0.5)),
    }

def reference(x, k_cache, v_cache, wq, wo):
    B, Sq, D = x.shape
    Hq, Dh = 32, 128
    Hkv = k_cache.shape[1]
    rep = Hq // Hkv
    q = (lambda x, *d: x.transpose(*d))((x @ wq).reshape(B, Sq, Hq, Dh), 0, 2, 1, 3)
    k = jnp.repeat(k_cache, rep, axis=1)
    v = jnp.repeat(v_cache, rep, axis=1)
    scores = jnp.einsum("bhqd,bhkd->bhqk", q, k) * (Dh ** -0.5)
    p = _softmax(scores, axis=-1)
    o = jnp.einsum("bhqk,bhkd->bhqd", p, v)
    return (lambda x, *d: x.transpose(*d))(o, 0, 2, 1, 3).reshape(B, Sq, Hq * Dh) @ wo
```

```python
import functools

import jax
import jax.numpy as jnp
import jax.experimental.pallas as pl
import jax.experimental.pallas.tpu as pltpu

_HQ = 32
_DH = 128


def _gqa_kernel(x_ref, k_ref, v_ref, wq_ref, wo_ref, o_ref, acc_ref, *, B, Sq, rep, Dh):
    g = pl.program_id(0)
    scale = Dh ** -0.5
    x = x_ref[...]
    q = jnp.dot(x, wq_ref[...], preferred_element_type=jnp.float32).astype(jnp.bfloat16)
    o_rows = []
    for b in range(B):
        qb = q[b * Sq:(b + 1) * Sq, :]
        qs = jnp.concatenate([qb[:, h * Dh:(h + 1) * Dh] for h in range(rep)], axis=0)
        k = k_ref[b, 0]
        v = v_ref[b, 0]
        s = jax.lax.dot_general(qs, k, (((1,), (1,)), ((), ())),
                                preferred_element_type=jnp.float32) * scale
        m = jnp.max(s, axis=-1, keepdims=True)
        e = jnp.exp(s - m)
        l = jnp.sum(e, axis=-1, keepdims=True)
        p = (e / l).astype(jnp.bfloat16)
        o = jnp.dot(p, v, preferred_element_type=jnp.float32).astype(jnp.bfloat16)
        o_rows.append(jnp.concatenate([o[h * Sq:(h + 1) * Sq, :] for h in range(rep)], axis=1))
    o_all = jnp.concatenate(o_rows, axis=0)
    part = jnp.dot(o_all, wo_ref[...], preferred_element_type=jnp.float32)

    @pl.when(g == 0)
    def _():
        acc_ref[...] = part

    @pl.when(g > 0)
    def _():
        acc_ref[...] += part

    @pl.when(g == pl.num_programs(0) - 1)
    def _():
        o_ref[...] = acc_ref[...].astype(o_ref.dtype)


@jax.jit
def pallas_standalone__gqa_block_cached__near_ridge_kernel(
    x: jax.Array,
    k_cache: jax.Array,
    v_cache: jax.Array,
    wq: jax.Array,
    wo: jax.Array,
):
    B, Sq, D = x.shape
    Hq, Dh = _HQ, _DH
    Hkv, Sk = k_cache.shape[1], k_cache.shape[2]
    rep = Hq // Hkv
    x2 = x.reshape(B * Sq, D)
    kern = functools.partial(_gqa_kernel, B=B, Sq=Sq, rep=rep, Dh=Dh)
    out = pl.pallas_call(
        kern,
        grid=(Hkv,),
        in_specs=[
            pl.BlockSpec((B * Sq, D), lambda g: (0, 0)),
            pl.BlockSpec((B, 1, Sk, Dh), lambda g: (0, g, 0, 0)),
            pl.BlockSpec((B, 1, Sk, Dh), lambda g: (0, g, 0, 0)),
            pl.BlockSpec((D, rep * Dh), lambda g: (0, g)),
            pl.BlockSpec((rep * Dh, D), lambda g: (g, 0)),
        ],
        out_specs=pl.BlockSpec((B * Sq, D), lambda g: (0, 0)),
        out_shape=jax.ShapeDtypeStruct((B * Sq, D), x.dtype),
        scratch_shapes=[pltpu.VMEM((B * Sq, D), jnp.float32)],
        compiler_params=pltpu.CompilerParams(dimension_semantics=("arbitrary",)),
    )(x2, k_cache, v_cache, wq, wo)
    return out.reshape(B, Sq, D)
```

```python
import functools

import jax
import jax.numpy as jnp
import jax.experimental.pallas as pl
import jax.experimental.pallas.tpu as pltpu

_HQ = 32
_DH = 128
_LOG2E = 1.4426950408889634

_ORDER = ("Q0 S0 S1 O0 S2 S3 Q1 P0 P1 S4 S5 O1 P2 P3 S6 S7 Q2 P4 P5 O2 P6 P7 Q3 O3").split()

_GROUPS = {
    "a": [("x", 0, 256), ("q", 0, 2)],
    "b": [("x", 256, 512)],
    "b2": [("q", 2, 4)],
    "c1": [("q", 4, 6)],
    "c2": [("k", 0, 1), ("v", 0, 1)],
    "c3": [("q", 6, 8)],
    "e": [("q", 8, 12)],
    "f": [("k", 1, 2), ("v", 1, 2), ("o", 0, 1)],
    "g": [("q", 12, 16), ("k", 2, 3), ("v", 2, 3), ("o", 1, 2)],
    "h": [("q", 16, 20), ("k", 3, 4), ("v", 3, 4), ("o", 2, 3)],
    "i": [("q", 20, 24), ("k", 4, 5), ("v", 4, 5), ("o", 3, 4)],
    "j": [("q", 24, 28), ("k", 5, 6), ("v", 5, 6), ("o", 4, 5)],
    "l": [("q", 28, 32), ("k", 6, 7), ("v", 6, 7), ("o", 5, 6)],
    "m": [("k", 7, 8), ("v", 7, 8), ("o", 6, 8)],
}
_HEAD = [
    ("+", "a"), ("+", "b"), ("+", "b2"), ("+", "c1"), ("+", "c2"), ("+", "c3"),
    ("?", "a"), ("Q", 0, 0, 256, None), ("Q", 1, 0, 256, 128), ("+", "e"),
    ("?", "b"), ("Q", 0, 256, 512, None), ("Q", 1, 256, 512, 48), ("+", "f"),
    ("?", "b2"), ("Q", 2, 0, 512, None), ("Q", 3, 0, 512, None),
]
_START = {(1, 1): ["g"], (2, 0): ["h"], (3, 0): ["i"], (4, 0): ["j"], (5, 0): ["l"], (6, 0): ["m"]}
_WAIT = {(1, 0): ["c1"], (1, 1): ["c2"], (1, 16): ["c3"], (2, 0): ["e"], (2, 1): ["f"], (3, 0): ["g"],
         (4, 0): ["h"], (5, 0): ["i"], (6, 0): ["j"], (7, 0): ["l"], (8, 0): ["m"]}
_NSEM = 6
_TAIL_SPLIT = 4


def _kernel(x_hbm, k_hbm, v_hbm, wq_hbm, wo_hbm, o_hbm,
            x_s, wq_s, wo_s, k_s, v_s, q_s0, q_s1, q_first, o_s0, o_s1, acc, out_s, sems,
            *, B, Sq, G, R, Dh, D):
    T = B * Sq
    NK = D // 128
    GW = R * Dh
    NT = G + 2
    bf, u32 = jnp.bfloat16, jnp.uint32
    c_exp = (Dh ** -0.5) * _LOG2E
    q_bufs = (q_s0, q_s1)
    o_bufs = (o_s0, o_s1)
    x_hbm, k_hbm, v_hbm, wq_hbm, wo_hbm = (r.bitcast(u32) for r in (x_hbm, k_hbm, v_hbm, wq_hbm, wo_hbm))

    def ld(w):
        return pltpu.bitcast(w, bf)

    def st(v):
        return pltpu.bitcast(v, u32)

    sem_of, busy = {}, set()

    def alloc(name):
        i = min(set(range(_NSEM)) - busy)
        busy.add(i)
        sem_of[name] = i

    def copies(name):
        sem = sems.at[sem_of[name]]
        out = []
        for kind, lo, hi in _GROUPS[name]:
            if kind == "x":
                sl = pl.ds(lo // 2, (hi - lo) // 2)
                out.append(pltpu.make_async_copy(x_hbm.at[sl, :], x_s.at[sl, :], sem))
            elif kind == "q":
                h = lo
                while h < hi:
                    g = h // R
                    e = min(hi, (g + 1) * R)
                    out.append(pltpu.make_async_copy(
                        wq_hbm.at[:, pl.ds(h * Dh, (e - h) * Dh)],
                        wq_s.at[g, :, pl.ds((h - g * R) * Dh, (e - h) * Dh)], sem))
                    h = e
            elif kind == "k":
                sl = pl.ds(lo, hi - lo)
                out.append(pltpu.make_async_copy(k_hbm.at[:, sl], k_s.at[:, sl], sem))
            elif kind == "v":
                sl = pl.ds(lo, hi - lo)
                out.append(pltpu.make_async_copy(v_hbm.at[:, sl], v_s.at[:, sl], sem))
            else:
                sl = pl.ds(lo * GW // 2, (hi - lo) * GW // 2)
                out.append(pltpu.make_async_copy(wo_hbm.at[sl, :], wo_s.at[sl, :], sem))
        return out

    started, waited = set(), set()

    def start(name):
        alloc(name)
        started.add(name)
        for d in copies(name):
            d.start()

    def wait(name):
        for d in copies(name):
            d.wait()
        waited.add(name)
        busy.discard(sem_of[name])

    out_pieces = []

    def out_copy(n, r0, r1):
        rs, cs = pl.ds(r0, r1 - r0), pl.ds(n * 128, 128)
        return pltpu.make_async_copy(out_s.at[rs, cs], o_hbm.at[rs, cs], sems.at[sem_of["out"]])

    deferred = []

    def qproj(h, r0=0, r1=T, pin=None):
        g, r = divmod(h, R)
        rs = pl.ds(r0 // 2, (r1 - r0) // 2)
        q = jnp.dot(ld(x_s[rs, :]), ld(wq_s[g, :, pl.ds(r * Dh, Dh)]),
                    preferred_element_type=jnp.float32).astype(bf)

        def store(a, e):
            if g == 0:
                q_first[r, pl.ds(r0 + a, e - a), :] = q[a:e]
            else:
                q_bufs[g % 2][r, pl.ds((r0 + a) // 2, (e - a) // 2), :] = st(q[a:e])

        if pin is None:
            store(0, r1 - r0)
        else:
            store(0, pin)
            deferred.append(lambda: store(pin, r1 - r0))

    def scores(g, b):
        if g == 0:
            qs = jnp.concatenate([q_first[r, pl.ds(b * Sq, Sq), :] for r in range(R)], axis=0)
        else:
            qb = q_bufs[g % 2]
            qs = ld(jnp.concatenate([qb[r, pl.ds(b * Sq // 2, Sq // 2), :] for r in range(R)], axis=0))
        s = jax.lax.dot_general(ld(k_s[b, g]), qs, (((1,), (1,)), ((), ())),
                                preferred_element_type=jnp.float32)
        m = jnp.max(s, axis=0, keepdims=True)
        e = jnp.exp2((s - m) * c_exp)
        l = jnp.sum(e, axis=0, keepdims=True)
        r = pl.reciprocal(l, approx=True)
        r = r * (2.0 - l * r)
        return (e * r).astype(bf).T

    def pv(g, b, p):
        o = st(jnp.dot(p, ld(v_s[b, g]), preferred_element_type=jnp.float32).astype(bf))
        ob = o_bufs[g % 2]
        for r in range(R):
            ob[r, pl.ds(b * Sq // 2, Sq // 2), :] = o[r * Sq // 2:(r + 1) * Sq // 2, :]

    def oproj(g, n, r0=0, r1=T):
        rs = pl.ds(r0, r1 - r0)
        rh = pl.ds(r0 // 2, (r1 - r0) // 2)
        ob = o_bufs[g % 2]
        o = ld(jnp.concatenate([ob[r, rh, :] for r in range(R)], axis=1))
        part = jnp.dot(o, ld(wo_s[pl.ds(g * GW // 2, GW // 2), pl.ds(n * 128, 128)]),
                       preferred_element_type=jnp.float32)
        if g == 0:
            acc[n, rs, :] = part
        elif g < G - 1:
            acc[n, rs, :] = acc[n, rs, :] + part
        else:
            out_s[rs, pl.ds(n * 128, 128)] = (acc[n, rs, :] + part).astype(out_s.dtype)
            if "out" not in sem_of:
                alloc("out")
            out_copy(n, r0, r1).start()
            out_pieces.append((n, r0, r1))

    for tok in _HEAD:
        if tok[0] == "+":
            start(tok[1])
        elif tok[0] == "?":
            wait(tok[1])
            while deferred:
                deferred.pop(0)()
        else:
            qproj(*tok[1:])

    for t in range(1, NT):
        gq, ga, go = t, t - 1, t - 2
        probs = {}
        for pos, op in enumerate(_ORDER):
            for name in _WAIT.get((t, pos), []):
                wait(name)
            for name in _START.get((t, pos), []):
                start(name)
            kind, i = op[0], int(op[1:])
            if kind == "S" and 0 <= ga < G:
                probs[i] = scores(ga, i)
            elif kind == "P" and 0 <= ga < G:
                pv(ga, i, probs.pop(i))
            elif kind == "Q" and gq < G:
                qproj(gq * R + i)
            elif kind == "O" and 0 <= go < G:
                if go == G - 1 and i == NK - 1:
                    c = T // _TAIL_SPLIT
                    for j in range(_TAIL_SPLIT):
                        oproj(go, i, j * c, (j + 1) * c)
                else:
                    oproj(go, i)

    assert started == waited == set(_GROUPS)
    for n, r0, r1 in out_pieces:
        out_copy(n, r0, r1).wait()


@jax.jit
def pallas_standalone__gqa_block_cached__near_ridge_kernel(
    x: jax.Array,
    k_cache: jax.Array,
    v_cache: jax.Array,
    wq: jax.Array,
    wo: jax.Array,
):
    B, Sq, D = x.shape
    Hq, Dh = _HQ, _DH
    G, Sk = k_cache.shape[1], k_cache.shape[2]
    R = Hq // G
    T = B * Sq
    NK = D // 128
    assert (B, NK, G, R) == (8, 4, 8, 4), "the static schedule is written for this problem size"
    bf, u32 = jnp.bfloat16, jnp.uint32
    packed = pltpu.VMEM((R, T // 2, Dh), u32)
    out = pl.pallas_call(
        functools.partial(_kernel, B=B, Sq=Sq, G=G, R=R, Dh=Dh, D=D),
        in_specs=[pl.BlockSpec(memory_space=pl.ANY)] * 5,
        out_specs=pl.BlockSpec(memory_space=pl.ANY),
        out_shape=jax.ShapeDtypeStruct((T, D), x.dtype),
        scratch_shapes=[
            pltpu.VMEM((T // 2, D), u32),
            pltpu.VMEM((G, D // 2, R * Dh), u32),
            pltpu.VMEM((Hq * Dh // 2, D), u32),
            pltpu.VMEM((B, G, Sk // 2, Dh), u32),
            pltpu.VMEM((B, G, Sk // 2, Dh), u32),
            packed, packed,
            pltpu.VMEM((R, T, Dh), bf),
            packed, packed,
            pltpu.VMEM((NK, T, 128), jnp.float32),
            pltpu.VMEM((T, D), bf),
            pltpu.SemaphoreType.DMA((_NSEM,)),
        ],
        compiler_params=pltpu.CompilerParams(
            vmem_limit_bytes=64 * 1024 * 1024,
            flags={"XLA_TPU_RESCHEDULE_DMA_DONES": True},
        ),
    )(x.reshape(T, D), k_cache, v_cache, wq, wo)
    return out.reshape(B, Sq, D)
```

```python
import jax
import jax.numpy as jnp
import jax.experimental.pallas as pl
import jax.experimental.pallas.tpu as pltpu

_HQ = 32
_DH = 128
_LOG2E = 1.4426950408889634

_LAG_A = 2
_LAG_O = 3
_HEAD_GROUPS = 2

_ORDER = "Q0 S0 S1 O0 S2 S3 Q1 P0 P1 S4 S5 O1 P2 P3 S6 S7 Q2 P4 P5 O2 P6 P7 Q3 O3".split()
_ORDER_FIRST = "Q0 S0 S1 S2 S3 Q1 P0 P1 S4 S5 P2 P3 Q2 S6 S7 P4 P5 Q3 P6 P7".split()

_GROUPS = {
    "a": [("qk0", 0, 1), ("x0", 0, 256)],
    "a1": [("x0", 256, 512)],
    "a2": [("qk1", 0, 1)],
    "b1": [("qk0", 1, 2), ("xs", 1, 2)],
    "b1b": [("qk1", 1, 2)],
    "b2": [("qk0", 2, 3), ("xs", 2, 3)],
    "b2b": [("qk1", 2, 3)],
    "b3": [("qk0", 3, 4), ("xs", 3, 4), ("qk1", 3, 4)],
    "d1": [("q", 8, 10)],
    "d2": [("k", 0, 1), ("v", 0, 1)],
    "d3": [("q", 10, 12)],
    "e1": [("q", 12, 14), ("k", 1, 2)],
    "e2": [("o", 0, 1)],
    "e3": [("v", 1, 2), ("q", 14, 16)],
    "f": [("q", 16, 20), ("k", 2, 3), ("v", 2, 3), ("o", 1, 2)],
    "g": [("q", 20, 24), ("k", 3, 4), ("v", 3, 4), ("o", 2, 3)],
    "h": [("q", 24, 28), ("k", 4, 5), ("v", 4, 5), ("o", 3, 4)],
    "i": [("q", 28, 32), ("k", 5, 6), ("v", 5, 6), ("o", 4, 5)],
    "j": [("k", 6, 7), ("v", 6, 7), ("o", 5, 6)],
    "l": [("k", 7, 8), ("v", 7, 8), ("o", 6, 8)],
}
_HEAD = [
    ("+", "a"), ("+", "a1"), ("+", "a2"), ("+", "b1"), ("+", "b1b"), ("+", "b2"), ("+", "b2b"), ("+", "b3"),
    ("?", "a"), ("K", 0, 0, 0, 256, 64), ("+", "d1"),
    ("?", "a1"), ("K", 0, 0, 256, 512, 64), ("+", "d2"),
    ("?", "a2"), ("K", 1, 0, 0, 512, 320), ("+", "d3"),
    ("?", "b1"), ("K", 0, 1, 0, 512, 64), ("+", "e1"),
    ("?", "b1b"), ("K", 1, 1, 0, 512, 320), ("+", "e2"),
    ("?", "b2"), ("K", 0, 2, 0, 512, 64), ("+", "e3"),
    ("?", "b2b"), ("K", 1, 2, 0, 512, 320), ("+", "f"),
    ("?", "b3"), ("K", 0, 3, 0, 512, None), ("K", 1, 3, 0, 512, 320), ("+", "g"),
    ("?", "d1"),
]
_START = {(4, 0): ["h"], (5, 0): ["i"], (6, 0): ["j"], (7, 0): ["l"]}
_WAIT = {(2, 1): ["d2"], (2, 12): ["d3"], (3, 0): ["e1"], (3, 3): ["e2"], (3, 7): ["e3"],
         (4, 0): ["f"], (5, 0): ["g"], (6, 0): ["h"], (7, 0): ["i"], (8, 0): ["j"], (9, 0): ["l"]}
_TAIL_SPLIT = 8


def _kernel(x_hbm, k_hbm, v_hbm, wq_hbm, wo_hbm, o_hbm,
            x_s, wq_s, wo_s, k_s, v_s, q_h0, q_h1, q_s0, q_s1, q_s2, o_s0, o_s1, acc, out_s,
            *, sems, B, Sq, G, R, Dh, D):
    T = B * Sq
    NK = D // 128
    GW = R * Dh
    bf, u32 = jnp.bfloat16, jnp.uint32
    c_exp = (Dh ** -0.5) * _LOG2E
    q_head = (q_h0, q_h1)
    q_bufs = (q_s0, q_s1, q_s2)
    o_bufs = (o_s0, o_s1)
    x_hbm, k_hbm, v_hbm, wq_hbm, wo_hbm = (r.bitcast(u32) for r in (x_hbm, k_hbm, v_hbm, wq_hbm, wo_hbm))

    def ld(w):
        return pltpu.bitcast(w, bf)

    def st(v):
        return pltpu.bitcast(v, u32)

    sem_of = {name: i for i, name in enumerate(_GROUPS)}
    out_sem = sems.at[len(_GROUPS)]

    def copies(name):
        sem = sems.at[sem_of[name]]
        out = []
        for kind, lo, hi in _GROUPS[name]:
            if kind == "x0":
                sl = pl.ds(lo // 2, (hi - lo) // 2)
                out.append(pltpu.make_async_copy(x_hbm.at[sl, pl.ds(0, 128)], x_s.at[sl, pl.ds(0, 128)], sem))
            elif kind == "xs":
                sl = pl.ds(lo * 128, (hi - lo) * 128)
                out.append(pltpu.make_async_copy(x_hbm.at[:, sl], x_s.at[:, sl], sem))
            elif kind in ("qk0", "qk1"):
                g = int(kind[2])
                sl = pl.ds(lo * 64, (hi - lo) * 64)
                out.append(pltpu.make_async_copy(wq_hbm.at[sl, pl.ds(g * GW, GW)], wq_s.at[g, sl, :], sem))
            elif kind == "q":
                h = lo
                while h < hi:
                    g = h // R
                    e = min(hi, (g + 1) * R)
                    out.append(pltpu.make_async_copy(
                        wq_hbm.at[:, pl.ds(h * Dh, (e - h) * Dh)],
                        wq_s.at[g, :, pl.ds((h - g * R) * Dh, (e - h) * Dh)], sem))
                    h = e
            elif kind == "k":
                sl = pl.ds(lo, hi - lo)
                out.append(pltpu.make_async_copy(k_hbm.at[:, sl], k_s.at[:, sl], sem))
            elif kind == "v":
                sl = pl.ds(lo, hi - lo)
                out.append(pltpu.make_async_copy(v_hbm.at[:, sl], v_s.at[:, sl], sem))
            else:
                sl = pl.ds(lo * GW // 2, (hi - lo) * GW // 2)
                out.append(pltpu.make_async_copy(wo_hbm.at[sl, :], wo_s.at[sl, :], sem))
        return out

    started, waited = set(), set()

    def start(name):
        started.add(name)
        for d in copies(name):
            d.start()

    def wait(name):
        assert name in started
        for d in copies(name):
            d.wait()
        waited.add(name)

    out_pieces = []

    def out_copy(n, r0, r1):
        rs, cs = pl.ds(r0, r1 - r0), pl.ds(n * 128, 128)
        return pltpu.make_async_copy(out_s.at[rs, cs], o_hbm.at[rs, cs], out_sem)

    deferred = []
    partial = {g: [] for g in range(_HEAD_GROUPS)}

    def qproj_ktile(g, kk, r0, r1, pin):
        part = jnp.dot(ld(x_s[pl.ds(r0 // 2, (r1 - r0) // 2), pl.ds(kk * 128, 128)]),
                       ld(wq_s[g, pl.ds(kk * 64, 64), :]),
                       preferred_element_type=jnp.float32)
        if kk == 0:
            tot = part
            partial[g].append(part)
        else:
            prev = partial[g][0] if len(partial[g]) == 1 else jnp.concatenate(partial[g], axis=0)
            tot = prev + part
            partial[g] = [tot]
        ref = q_head[g]
        if kk < NK - 1:
            if pin is not None:
                ref[0, pl.ds(r0 + pin, 16), :] = tot[pin:pin + 16, 0:Dh].astype(bf)
            return
        q = tot.astype(bf)

        def store(a, e):
            for r in range(R):
                ref[r, pl.ds(a, e - a), :] = q[a:e, r * Dh:(r + 1) * Dh]

        if pin is None:
            store(0, T)
        else:
            store(0, pin)
            deferred.append(lambda: store(pin, T))

    def qproj(h):
        g, r = divmod(h, R)
        q = jnp.dot(ld(x_s[...]), ld(wq_s[g, :, pl.ds(r * Dh, Dh)]),
                    preferred_element_type=jnp.float32).astype(bf)
        q_bufs[g % 3][r] = st(q)

    def scores(g, b):
        if g < _HEAD_GROUPS:
            qb = q_head[g]
            qs = jnp.concatenate([qb[r, pl.ds(b * Sq, Sq), :] for r in range(R)], axis=0)
        else:
            qb = q_bufs[g % 3]
            qs = ld(jnp.concatenate([qb[r, pl.ds(b * Sq // 2, Sq // 2), :] for r in range(R)], axis=0))
        s = jax.lax.dot_general(ld(k_s[b, g]), qs, (((1,), (1,)), ((), ())),
                                preferred_element_type=jnp.float32)
        m = jnp.max(s, axis=0, keepdims=True)
        e = jnp.exp2((s - m) * c_exp)
        l = jnp.sum(e, axis=0, keepdims=True)
        r = pl.reciprocal(l, approx=True)
        r = r * (2.0 - l * r)
        return (e * r).astype(bf).T

    def pv(g, b, p):
        o = st(jnp.dot(p, ld(v_s[b, g]), preferred_element_type=jnp.float32).astype(bf))
        ob = o_bufs[g % 2]
        for r in range(R):
            ob[r, pl.ds(b * Sq // 2, Sq // 2), :] = o[r * Sq // 2:(r + 1) * Sq // 2, :]

    def oproj(g, n, r0=0, r1=T):
        rs = pl.ds(r0, r1 - r0)
        rh = pl.ds(r0 // 2, (r1 - r0) // 2)
        ob = o_bufs[g % 2]
        o = ld(jnp.concatenate([ob[r, rh, :] for r in range(R)], axis=1))
        part = jnp.dot(o, ld(wo_s[pl.ds(g * GW // 2, GW // 2), pl.ds(n * 128, 128)]),
                       preferred_element_type=jnp.float32)
        if g == 0:
            acc[n, rs, :] = part
        elif g < G - 1:
            acc[n, rs, :] = acc[n, rs, :] + part
        else:
            out_s[rs, pl.ds(n * 128, 128)] = (acc[n, rs, :] + part).astype(out_s.dtype)
            out_copy(n, r0, r1).start()
            out_pieces.append((n, r0, r1))

    for tok in _HEAD:
        if tok[0] == "+":
            start(tok[1])
        elif tok[0] == "?":
            wait(tok[1])
            while deferred:
                deferred.pop(0)()
        else:
            qproj_ktile(*tok[1:])
    assert not deferred

    for t in range(_HEAD_GROUPS, G + _LAG_O):
        gq, ga, go = t, t - _LAG_A, t - _LAG_O
        probs = {}
        for pos, op in enumerate(_ORDER_FIRST if t == _LAG_A else _ORDER):
            for name in _WAIT.get((t, pos), []):
                wait(name)
            for name in _START.get((t, pos), []):
                start(name)
            kind, i = op[0], int(op[1:])
            if kind == "S" and 0 <= ga < G:
                probs[i] = scores(ga, i)
            elif kind == "P" and 0 <= ga < G:
                pv(ga, i, probs.pop(i))
            elif kind == "Q" and gq < G:
                qproj(gq * R + i)
            elif kind == "O" and 0 <= go < G:
                if go == G - 1 and i == NK - 1:
                    c = T // _TAIL_SPLIT
                    for j in range(_TAIL_SPLIT):
                        oproj(go, i, j * c, (j + 1) * c)
                else:
                    oproj(go, i)

    assert started == waited == set(_GROUPS)
    for n, r0, r1 in out_pieces:
        out_copy(n, r0, r1).wait()


@jax.jit
def pallas_standalone__gqa_block_cached__near_ridge_kernel(
    x: jax.Array,
    k_cache: jax.Array,
    v_cache: jax.Array,
    wq: jax.Array,
    wo: jax.Array,
):
    B, Sq, D = x.shape
    Hq, Dh = _HQ, _DH
    G, Sk = k_cache.shape[1], k_cache.shape[2]
    R = Hq // G
    T = B * Sq
    NK = D // 128
    assert (B, Sq, NK, G, R) == (8, 64, 4, 8, 4), "the static schedule is written for this problem size"
    bf, u32 = jnp.bfloat16, jnp.uint32
    plain = pltpu.VMEM((R, T, Dh), bf)
    packed = pltpu.VMEM((R, T // 2, Dh), u32)

    def kernel(*refs):
        pl.run_scoped(
            lambda sems: _kernel(*refs, sems=sems, B=B, Sq=Sq, G=G, R=R, Dh=Dh, D=D),
            pltpu.SemaphoreType.DMA((len(_GROUPS) + 1,)))

    out = pl.pallas_call(
        kernel,
        in_specs=[pl.BlockSpec(memory_space=pl.ANY)] * 5,
        out_specs=pl.BlockSpec(memory_space=pl.ANY),
        out_shape=jax.ShapeDtypeStruct((T, D), x.dtype),
        scratch_shapes=[
            pltpu.VMEM((T // 2, D), u32),
            pltpu.VMEM((G, D // 2, R * Dh), u32),
            pltpu.VMEM((Hq * Dh // 2, D), u32),
            pltpu.VMEM((B, G, Sk // 2, Dh), u32),
            pltpu.VMEM((B, G, Sk // 2, Dh), u32),
            plain, plain,
            packed, packed, packed,
            packed, packed,
            pltpu.VMEM((NK, T, 128), jnp.float32),
            pltpu.VMEM((T, D), bf),
        ],
        compiler_params=pltpu.CompilerParams(
            vmem_limit_bytes=64 * 1024 * 1024,
            flags={"XLA_TPU_RESCHEDULE_DMA_DONES": True},
        ),
    )(x.reshape(T, D), k_cache, v_cache, wq, wo)
    return out.reshape(B, Sq, D)
```

```python
import jax
import jax.numpy as jnp
import jax.experimental.pallas as pl
import jax.experimental.pallas.tpu as pltpu

_HQ = 32
_DH = 128
_LOG2E = 1.4426950408889634

_LAG_A = 2
_LAG_O = 3
_HEAD_GROUPS = 2

_ORDER = "Q0 S0 S1 O0 S2 S3 Q1 P0 P1 S4 S5 O1 P2 P3 S6 S7 Q2 P4 P5 O2 P6 P7 Q3 O3".split()
_ORDER_FIRST = "Q0 S0 S1 S2 S3 Q1 P0 P1 S4 S5 P2 P3 Q2 S6 S7 P4 P5 Q3 P6 P7".split()

_GROUPS = {
    "a": [("qk0", 0, 1), ("x0", 0, 192)],
    "a1": [("x0", 192, 512)],
    "a2": [("qk1", 0, 1)],
    "b1": [("qk0", 1, 2), ("xs", 1, 2)],
    "b1b": [("qk1", 1, 2)],
    "b2": [("qk0", 2, 3), ("xs", 2, 3)],
    "b2b": [("qk1", 2, 3)],
    "b3": [("qk0", 3, 4), ("xs", 3, 4), ("qk1", 3, 4)],
    "d1": [("q", 8, 10)],
    "d2": [("k", 0, 1), ("v", 0, 1)],
    "d3": [("q", 10, 12)],
    "e1": [("q", 12, 14), ("k", 1, 2)],
    "e2": [("o", 0, 1)],
    "e3": [("v", 1, 2), ("q", 14, 16)],
    "f": [("q", 16, 20), ("k", 2, 3), ("v", 2, 3), ("o", 1, 2)],
    "g": [("q", 20, 24), ("k", 3, 4), ("v", 3, 4), ("o", 2, 3)],
    "h": [("q", 24, 28), ("k", 4, 5), ("v", 4, 5), ("o", 3, 4)],
    "i": [("q", 28, 32), ("k", 5, 6), ("v", 5, 6), ("o", 4, 5)],
    "j": [("k", 6, 7), ("v", 6, 7), ("o", 5, 6)],
    "l": [("k", 7, 8), ("v", 7, 8), ("o", 6, 8)],
}
_HEAD = [
    ("+", "a"), ("+", "a1"), ("+", "a2"), ("+", "b1"), ("+", "b1b"), ("+", "b2"), ("+", "b2b"), ("+", "b3"),
    ("?", "a"), ("K", 0, 0, 0, 192, 16), ("+", "d1"),
    ("?", "a1"), ("K", 0, 0, 192, 512, 128), ("+", "d2"),
    ("?", "a2"), ("K", 1, 0, 0, 512, 320), ("+", "d3"),
    ("?", "b1"), ("K", 0, 1, 0, 512, 64), ("+", "e1"),
    ("?", "b1b"), ("K", 1, 1, 0, 512, 320), ("+", "e2"),
    ("?", "b2"), ("K", 0, 2, 0, 512, 64), ("+", "e3"),
    ("?", "b2b"), ("K", 1, 2, 0, 512, 320), ("+", "f"),
    ("?", "b3"), ("K", 0, 3, 0, 512, None), ("K", 1, 3, 0, 512, 320), ("+", "g"),
    ("?", "d1"),
]
_START = {(4, 0): ["h"], (5, 0): ["i"], (6, 0): ["j"], (7, 0): ["l"]}
_WAIT = {(2, 1): ["d2"], (2, 12): ["d3"], (3, 0): ["e1"], (3, 3): ["e2"], (3, 7): ["e3"],
         (4, 0): ["f"], (5, 0): ["g"], (6, 0): ["h"], (7, 0): ["i"], (8, 0): ["j"], (9, 0): ["l"]}
_TAIL_SPLIT = 8


def _kernel(x_hbm, k_hbm, v_hbm, wq_hbm, wo_hbm, o_hbm,
            x_s, wq_s, wo_s, k_s, v_s, q_h0, q_h1, q_s0, q_s1, q_s2, o_s0, o_s1, acc, out_s,
            *, sems, B, Sq, G, R, Dh, D):
    T = B * Sq
    NK = D // 128
    GW = R * Dh
    bf, u32 = jnp.bfloat16, jnp.uint32
    c_exp = (Dh ** -0.5) * _LOG2E
    q_head = (q_h0, q_h1)
    q_bufs = (q_s0, q_s1, q_s2)
    o_bufs = (o_s0, o_s1)
    x_hbm, k_hbm, v_hbm, wq_hbm, wo_hbm = (r.bitcast(u32) for r in (x_hbm, k_hbm, v_hbm, wq_hbm, wo_hbm))

    def ld(w):
        return pltpu.bitcast(w, bf)

    def st(v):
        return pltpu.bitcast(v, u32)

    sem_of = {name: i for i, name in enumerate(_GROUPS)}
    out_sem = sems.at[len(_GROUPS)]

    def copies(name):
        sem = sems.at[sem_of[name]]
        out = []
        for kind, lo, hi in _GROUPS[name]:
            if kind == "x0":
                sl = pl.ds(lo // 2, (hi - lo) // 2)
                out.append(pltpu.make_async_copy(x_hbm.at[sl, pl.ds(0, 128)], x_s.at[sl, pl.ds(0, 128)], sem))
            elif kind == "xs":
                sl = pl.ds(lo * 128, (hi - lo) * 128)
                out.append(pltpu.make_async_copy(x_hbm.at[:, sl], x_s.at[:, sl], sem))
            elif kind in ("qk0", "qk1"):
                g = int(kind[2])
                sl = pl.ds(lo * 64, (hi - lo) * 64)
                out.append(pltpu.make_async_copy(wq_hbm.at[sl, pl.ds(g * GW, GW)], wq_s.at[g, sl, :], sem))
            elif kind == "q":
                h = lo
                while h < hi:
                    g = h // R
                    e = min(hi, (g + 1) * R)
                    out.append(pltpu.make_async_copy(
                        wq_hbm.at[:, pl.ds(h * Dh, (e - h) * Dh)],
                        wq_s.at[g, :, pl.ds((h - g * R) * Dh, (e - h) * Dh)], sem))
                    h = e
            elif kind == "k":
                sl = pl.ds(lo, hi - lo)
                out.append(pltpu.make_async_copy(k_hbm.at[:, sl], k_s.at[:, sl], sem))
            elif kind == "v":
                sl = pl.ds(lo, hi - lo)
                out.append(pltpu.make_async_copy(v_hbm.at[:, sl], v_s.at[:, sl], sem))
            else:
                sl = pl.ds(lo * GW // 2, (hi - lo) * GW // 2)
                out.append(pltpu.make_async_copy(wo_hbm.at[sl, :], wo_s.at[sl, :], sem))
        return out

    started, waited = set(), set()

    def start(name):
        started.add(name)
        for d in copies(name):
            d.start()

    def wait(name):
        assert name in started
        for d in copies(name):
            d.wait()
        waited.add(name)

    out_pieces = []

    def out_copy(n, r0, r1):
        rs, cs = pl.ds(r0, r1 - r0), pl.ds(n * 128, 128)
        return pltpu.make_async_copy(out_s.at[rs, cs], o_hbm.at[rs, cs], out_sem)

    deferred = []
    partial = {g: [] for g in range(_HEAD_GROUPS)}

    def qproj_ktile(g, kk, r0, r1, pin):
        part = jnp.dot(ld(x_s[pl.ds(r0 // 2, (r1 - r0) // 2), pl.ds(kk * 128, 128)]),
                       ld(wq_s[g, pl.ds(kk * 64, 64), :]),
                       preferred_element_type=jnp.float32)
        if kk == 0:
            tot = part
            partial[g].append(part)
        else:
            prev = partial[g][0] if len(partial[g]) == 1 else jnp.concatenate(partial[g], axis=0)
            tot = prev + part
            partial[g] = [tot]
        ref = q_head[g]
        if kk < NK - 1:
            if pin is not None:
                ref[0, pl.ds(r0 + pin, 16), :] = tot[pin:pin + 16, 0:Dh].astype(bf)
            return
        q = tot.astype(bf)

        def store(a, e):
            for r in range(R):
                ref[r, pl.ds(a, e - a), :] = q[a:e, r * Dh:(r + 1) * Dh]

        if pin is None:
            store(0, T)
        else:
            store(0, pin)
            deferred.append(lambda: store(pin, T))

    def qproj(h):
        g, r = divmod(h, R)
        q = jnp.dot(ld(x_s[...]), ld(wq_s[g, :, pl.ds(r * Dh, Dh)]),
                    preferred_element_type=jnp.float32).astype(bf)
        q_bufs[g % 3][r] = st(q)

    def scores(g, b):
        if g < _HEAD_GROUPS:
            qb = q_head[g]
            qs = jnp.concatenate([qb[r, pl.ds(b * Sq, Sq), :] for r in range(R)], axis=0)
        else:
            qb = q_bufs[g % 3]
            qs = ld(jnp.concatenate([qb[r, pl.ds(b * Sq // 2, Sq // 2), :] for r in range(R)], axis=0))
        s = jax.lax.dot_general(ld(k_s[b, g]), qs, (((1,), (1,)), ((), ())),
                                preferred_element_type=jnp.float32)
        m = jnp.max(s, axis=0, keepdims=True)
        e = jnp.exp2((s - m) * c_exp)
        l = jnp.sum(e, axis=0, keepdims=True)
        r = pl.reciprocal(l, approx=True)
        r = r * (2.0 - l * r)
        return (e * r).astype(bf).T

    def pv(g, b, p):
        o = st(jnp.dot(p, ld(v_s[b, g]), preferred_element_type=jnp.float32).astype(bf))
        ob = o_bufs[g % 2]
        for r in range(R):
            ob[r, pl.ds(b * Sq // 2, Sq // 2), :] = o[r * Sq // 2:(r + 1) * Sq // 2, :]

    def oproj(g, n, r0=0, r1=T):
        rs = pl.ds(r0, r1 - r0)
        rh = pl.ds(r0 // 2, (r1 - r0) // 2)
        ob = o_bufs[g % 2]
        o = ld(jnp.concatenate([ob[r, rh, :] for r in range(R)], axis=1))
        part = jnp.dot(o, ld(wo_s[pl.ds(g * GW // 2, GW // 2), pl.ds(n * 128, 128)]),
                       preferred_element_type=jnp.float32)
        if g == 0:
            acc[n, rs, :] = part
        elif g < G - 1:
            acc[n, rs, :] = acc[n, rs, :] + part
        else:
            out_s[rs, pl.ds(n * 128, 128)] = (acc[n, rs, :] + part).astype(out_s.dtype)
            out_copy(n, r0, r1).start()
            out_pieces.append((n, r0, r1))

    for tok in _HEAD:
        if tok[0] == "+":
            start(tok[1])
        elif tok[0] == "?":
            wait(tok[1])
            while deferred:
                deferred.pop(0)()
        else:
            qproj_ktile(*tok[1:])
    assert not deferred

    for t in range(_HEAD_GROUPS, G + _LAG_O):
        gq, ga, go = t, t - _LAG_A, t - _LAG_O
        probs = {}
        for pos, op in enumerate(_ORDER_FIRST if t == _LAG_A else _ORDER):
            for name in _WAIT.get((t, pos), []):
                wait(name)
            for name in _START.get((t, pos), []):
                start(name)
            kind, i = op[0], int(op[1:])
            if kind == "S" and 0 <= ga < G:
                probs[i] = scores(ga, i)
            elif kind == "P" and 0 <= ga < G:
                pv(ga, i, probs.pop(i))
            elif kind == "Q" and gq < G:
                qproj(gq * R + i)
            elif kind == "O" and 0 <= go < G:
                if go == G - 1 and i == NK - 1:
                    c = T // _TAIL_SPLIT
                    for j in range(_TAIL_SPLIT):
                        oproj(go, i, j * c, (j + 1) * c)
                else:
                    oproj(go, i)

    assert started == waited == set(_GROUPS)
    for n, r0, r1 in out_pieces:
        out_copy(n, r0, r1).wait()


@jax.jit
def pallas_standalone__gqa_block_cached__near_ridge_kernel(
    x: jax.Array,
    k_cache: jax.Array,
    v_cache: jax.Array,
    wq: jax.Array,
    wo: jax.Array,
):
    B, Sq, D = x.shape
    Hq, Dh = _HQ, _DH
    G, Sk = k_cache.shape[1], k_cache.shape[2]
    R = Hq // G
    T = B * Sq
    NK = D // 128
    assert (B, Sq, NK, G, R) == (8, 64, 4, 8, 4), "the static schedule is written for this problem size"
    bf, u32 = jnp.bfloat16, jnp.uint32
    plain = pltpu.VMEM((R, T, Dh), bf)
    packed = pltpu.VMEM((R, T // 2, Dh), u32)

    def kernel(*refs):
        pl.run_scoped(
            lambda sems: _kernel(*refs, sems=sems, B=B, Sq=Sq, G=G, R=R, Dh=Dh, D=D),
            pltpu.SemaphoreType.DMA((len(_GROUPS) + 1,)))

    out = pl.pallas_call(
        kernel,
        in_specs=[pl.BlockSpec(memory_space=pl.ANY)] * 5,
        out_specs=pl.BlockSpec(memory_space=pl.ANY),
        out_shape=jax.ShapeDtypeStruct((T, D), x.dtype),
        scratch_shapes=[
            pltpu.VMEM((T // 2, D), u32),
            pltpu.VMEM((G, D // 2, R * Dh), u32),
            pltpu.VMEM((Hq * Dh // 2, D), u32),
            pltpu.VMEM((B, G, Sk // 2, Dh), u32),
            pltpu.VMEM((B, G, Sk // 2, Dh), u32),
            plain, plain,
            packed, packed, packed,
            packed, packed,
            pltpu.VMEM((NK, T, 128), jnp.float32),
            pltpu.VMEM((T, D), bf),
        ],
        compiler_params=pltpu.CompilerParams(
            vmem_limit_bytes=64 * 1024 * 1024,
            flags={"XLA_TPU_RESCHEDULE_DMA_DONES": True},
        ),
    )(x.reshape(T, D), k_cache, v_cache, wq, wo)
    return out.reshape(B, Sq, D)
```
